```python
import os as _os
_os.environ.setdefault("JAX_PLATFORMS", "cpu")
import jax
import jax.numpy as jnp

def _softmax(x, axis=-1):
    return jax.nn.softmax(x, axis=axis)
def _gelu(x):
    return jax.nn.gelu(x, approximate=True)
def _silu(x):
    return jax.nn.silu(x)
def _sigmoid(x):
    return jax.nn.sigmoid(x)
def _layernorm(x, axis=-1, eps=1e-5):
    m = jnp.mean(x, axis=axis, keepdims=True)
    v = jnp.var(x, axis=axis, keepdims=True)
    return (x - m) / jnp.sqrt(v + eps)
def _scatter_add(tgt, idx, src, axis=0):
    return tgt.at[idx].add(src)
def _segment_sum(src, seg, n):
    return jax.ops.segment_sum(src, seg, n)
class _Rng:
    def __init__(self, key):
        self._k = key
    def _next(self):
        self._k, sub = jax.random.split(self._k)
        return sub
    def normal(self, shape):
        return jax.random.normal(self._next(), shape, dtype=jnp.bfloat16)
    def randint(self, lo, hi, shape):
        return jax.random.randint(self._next(), shape, lo, hi, dtype=jnp.int32)
    def uniform(self, shape, lo=0.0, hi=1.0):
        return jax.random.uniform(self._next(), shape, jnp.bfloat16, lo, hi)
    def permutation(self, n):
        return jax.random.permutation(self._next(), n)


kernel_name = 'concat_heads__sliding_local_dilated__sliding_block__prompt'

def setup_inputs():
    _rng = _Rng(jax.random.key(int.from_bytes(__import__("os").urandom(4), "little")))
    _w = (lambda a: (lambda t: t.astype(jnp.bfloat16) if jnp.issubdtype(t.dtype, jnp.floating) else t)(jnp.asarray(a)))
    def _A_setup():
        B, S, D = 1, 2048, 1024
        return {
            "x": _w((lambda *s: _rng.normal(s) * 0.2)(B, S, D)),
            "wqkv": _w((lambda *s: _rng.normal(s) * 0.2)(D, 3 * D)),
            "wo": _w((lambda *s: _rng.normal(s) * 0.05)(D, D)),
        }
    _A_in = _A_setup()

    def _B_setup():
        B, S, D = 1, 2048, 1024
        return {
            "x": _w((lambda *s: _rng.normal(s) * 0.2)(B, S, D)),
            "wqkv": _w((lambda *s: _rng.normal(s) * 0.2)(D, 3 * D)),
            "wo": _w((lambda *s: _rng.normal(s) * 0.05)(D, D)),
        }
    _B_in = _B_setup()

    return {
        "A_x": _A_in["x"],
        "A_wqkv": _A_in["wqkv"],
        "A_wo": _A_in["wo"],
        "B_x": _B_in["x"],
        "B_wqkv": _B_in["wqkv"],
        "B_wo": _B_in["wo"],
    }

def reference(A_x, A_wqkv, A_wo, B_x, B_wqkv, B_wo):
    def _A_ref(x, wqkv, wo):
        B, S, D = x.shape
        H = 32; Dh = D // H
        W, dil = 8, 2
        qkv = (lambda x, *d: x.transpose(*d))((x @ wqkv).reshape(B, S, 3, H, Dh), 2, 0, 3, 1, 4)
        q, k, v = qkv[0], qkv[1], qkv[2]
        scale = Dh ** -0.5
        pos = jnp.arange(S)
        off = jnp.arange(W) * dil
        idx = pos[:, None] - off[None, :]
        mask = idx >= 0
        idx_c = jnp.where(mask, idx, 0).reshape(-1)
        kg = k[:, :, idx_c, :].reshape(B, H, S, W, Dh)
        vg = v[:, :, idx_c, :].reshape(B, H, S, W, Dh)
        logits = jnp.einsum("bhsd,bhswd->bhsw", q, kg) * scale
        logits = jnp.where(mask[None, None, :, :], logits, -1e9)
        attn = _softmax(logits, axis=-1)
        o = jnp.einsum("bhsw,bhswd->bhsd", attn, vg)
        return (lambda x, *d: x.transpose(*d))(o, 0, 2, 1, 3).reshape(B, S, D) @ wo

    def _B_ref(x, wqkv, wo):
        B, S, D = x.shape
        H = 32; Dh = D // H; W = 256
        qkv = (lambda x, *d: x.transpose(*d))((x @ wqkv).reshape(B, S, 3, H, Dh), 2, 0, 3, 1, 4)
        q, k, v = qkv[0], qkv[1], qkv[2]
        scores = jnp.einsum("bhqd,bhkd->bhqk", q, k) * (Dh ** -0.5)
        idx = jnp.arange(S)
        mask = (idx[:, None] - idx[None, :] >= 0) & (idx[:, None] - idx[None, :] < W)
        scores = jnp.where(mask[None, None], scores, -1e9)
        p = _softmax(scores, axis=-1)
        o = jnp.einsum("bhqk,bhkd->bhqd", p, v)
        return (lambda x, *d: x.transpose(*d))(o, 0, 2, 1, 3).reshape(B, S, D) @ wo

    a = _A_ref(A_x, A_wqkv, A_wo)
    b = _B_ref(B_x, B_wqkv, B_wo)
    return jnp.concatenate([a, b], axis=-1)
```

```python
import jax
import jax.numpy as jnp
from jax import lax
import jax.experimental.pallas as pl
import jax.experimental.pallas.tpu as pltpu

S = 2048
D = 1024
DH = 32
R = 256
NB = S // R
NG = D // 128
LOG2E = 1.4426950408889634
QSCALE = (DH ** -0.5) * LOG2E
NEG = -1e30
NSLOT = 3
LOOKAHEAD = 6
SCHED = "a"

BF = jnp.bfloat16
F32 = jnp.float32
U32 = jnp.uint32
NT = (((1,), (1,)), ((), ()))


def _dot(a, b):
    return jnp.dot(a, b, preferred_element_type=F32)


def _dot_nt(a, b):
    return lax.dot_general(a, b, NT, preferred_element_type=F32)


def _bf(x):
    return pltpu.bitcast(x, BF)


def _kernel(xa_hbm, wa_hbm, woa_hbm, xb_hbm, wb_hbm, wob_hbm, out_hbm,
            x_s, w_s, k_s, vt_s, q_s, o_s, out_s, zero_s, *rest):
    s_slots = rest[:NSLOT]
    in_sems, out_sems, zsem = rest[NSLOT:]
    x_hbm = (xa_hbm, xb_hbm)
    w_hbm = (wa_hbm, wb_hbm)
    wo_hbm = (woa_hbm, wob_hbm)

    copies = []
    index = {}

    def add(name, src, dst):
        index[name] = len(copies)
        copies.append(pltpu.make_async_copy(src, dst, in_sems.at[len(copies)]))

    def add_x(p, i):
        for k in range(8):
            add(("x", p, i, k), x_hbm[p].at[pl.ds(i * R, R), pl.ds(128 * k, 128)], x_s.at[p, i, k])

    def add_w(p, n):
        if n < 24:
            add(("w", p, n), w_hbm[p].at[:, pl.ds(128 * n, 128)], w_s.at[p, n])
        else:
            add(("w", p, n), wo_hbm[p].at[:, pl.ds(128 * (n - 24), 128)], w_s.at[p, n])

    add_x(0, 0)
    for n in range(24):
        add_w(0, n)
    add_x(1, 0)
    for g in range(NG):
        for j in range(3):
            add_w(1, 8 * j + g)
    for n in range(24, 32):
        add_w(0, n)
    if NB > 1:
        add_x(0, 1)
    for n in range(24, 32):
        add_w(1, n)
    if NB > 1:
        add_x(1, 1)
    for i in range(2, NB):
        add_x(0, i)
        add_x(1, i)

    state = {"started": 0, "waited": 0}

    def start_upto(n):
        n = min(n, len(copies))
        while state["started"] < n:
            copies[state["started"]].start()
            state["started"] += 1

    def need(name):
        j = index[name]
        start_upto(j + 1 + LOOKAHEAD)
        while state["waited"] <= j:
            copies[state["waited"]].wait()
            state["waited"] += 1

    start_upto(8 + 2 * LOOKAHEAD)

    xu = x_s.bitcast(U32)
    wu = w_s.bitcast(U32)
    ku = k_s.bitcast(U32)
    vtu = vt_s.bitcast(U32)
    qu = q_s.bitcast(U32)
    ou = o_s.bitcast(U32)

    zero_s[...] = jnp.zeros((8, 128), F32)
    z8 = pl.multiple_of(pl.semaphore_read(zsem), 8)
    zero_row = zero_s[pl.ds(z8, 8), :]

    def zeros_f32(r, c):
        return jnp.broadcast_to(zero_row[0:1, 0:1], (r, c))

    r128 = lax.broadcasted_iota(jnp.int32, (128, 512), 0)
    c128 = lax.broadcasted_iota(jnp.int32, (128, 512), 1) & 127
    upper = r128 > c128
    lane64 = lax.broadcasted_iota(jnp.int32, (64, 128), 1) >> 5

    def lhs_x(p, i):
        return jnp.concatenate([_bf(xu[p, i, k]) for k in range(8)], axis=1)

    def proj_tile(p, i, n):
        need(("w", p, n))
        for k in range(8):
            need(("x", p, i, k))
        return _dot(lhs_x(p, i), _bf(wu[p, n]))

    def proj_q(p, i, g):
        q_s[p, g] = (proj_tile(p, i, g) * QSCALE).astype(BF)

    def proj_k(p, i, g):
        k_s[p, g, i * R:(i + 1) * R, :] = proj_tile(p, i, 8 + g).astype(BF)

    def proj_v(p, i, g):
        v = proj_tile(p, i, 16 + g)
        for t in range(R // 128):
            vt_s[p, 2 * i + t, 128 * g:128 * g + 128, :] = v[128 * t:128 * t + 128].T.astype(BF)

    def out_tile(p, i, n):
        need(("w", p, 24 + n))
        lhs = jnp.concatenate([_bf(ou[p, g]) for g in range(NG)], axis=1)
        out_s[8 * p + n, i * R:(i + 1) * R, :] = _dot(lhs, _bf(wu[p, 24 + n])).astype(BF)
        cp = pltpu.make_async_copy(
            out_s.at[8 * p + n, pl.ds(i * R, R), :],
            out_hbm.at[pl.ds(i * R, R), pl.ds(D * p + 128 * n, 128)],
            out_sems.at[(i * 2 + p) * 8 + n])
        cp.start()
        return cp

    def qcat(p, g, t):
        qi = qu[p, g, 64 * t:64 * t + 64, :]
        return _bf(jnp.concatenate(
            [jnp.where(lane64 == h, qi, jnp.uint32(0)) for h in range(4)], axis=0))

    slot_ctr = {"n": 0}

    def next_slot():
        s = s_slots[slot_ctr["n"] % NSLOT]
        slot_ctr["n"] += 1
        return s

    def finish(p, g, t, outs, inv):
        o_t = jnp.concatenate(
            [outs[h] * inv[:, 128 * h:128 * h + 128] for h in range(4)], axis=0)
        o_s[p, g, 128 * t:128 * t + 128, :] = o_t.T.astype(BF)

    def recip(l):
        r0 = pl.reciprocal(l, approx=True)
        return r0 * (2.0 - l * r0)

    def b_qk(i, g, t):
        T = 2 * i + t
        s_ref = next_slot()
        if T >= 2:
            k0 = (T - 2) * 64
            parts = []
            for j in range(8):
                parts.append(ku[1, g, k0 + 8 * j:k0 + 8 * j + 8, :])
                parts.append(ku[1, g, k0 + 128 + 8 * j:k0 + 128 + 8 * j + 8, :])
            parts.append(ku[1, g, k0 + 64:k0 + 128, :])
            s = _dot_nt(_bf(jnp.concatenate(parts, axis=0)), qcat(1, g, t))
            s1 = jnp.concatenate([s[32 * j:32 * j + 16] for j in range(8)], axis=0)
            s3 = jnp.concatenate([s[32 * j + 16:32 * j + 32] for j in range(8)], axis=0)
            sm = jnp.where(upper, s1, s3)
            s2 = s[256:384]
            m = jnp.max(jnp.maximum(sm, s2), axis=0, keepdims=True)
            s_ref[0:128] = sm
            s_ref[128:256] = s2
        elif T == 1:
            s = _dot_nt(_bf(ku[1, g, 0:128, :]), qcat(1, g, t))
            sm = jnp.where(upper, NEG, s[128:256])
            s2 = s[0:128]
            m = jnp.max(jnp.maximum(sm, s2), axis=0, keepdims=True)
            s_ref[0:128] = sm
            s_ref[128:256] = s2
        else:
            s = _dot_nt(_bf(ku[1, g, 0:64, :]), qcat(1, g, t))
            sm = jnp.where(upper, NEG, s)
            m = jnp.max(sm, axis=0, keepdims=True)
            s_ref[0:128] = sm
        return s_ref, m

    def b_pv(i, g, t, st):
        s_ref, m = st
        T = 2 * i + t
        pm = jnp.exp2(s_ref[pl.ds(z8, 128)] - m)
        if T >= 1:
            p2 = jnp.exp2(s_ref[pl.ds(z8 + 128, 128)] - m)
            l = jnp.sum(pm + p2, axis=0, keepdims=True)
        else:
            l = jnp.sum(pm, axis=0, keepdims=True)
        inv = recip(l)
        if T >= 2:
            p1 = jnp.where(upper, pm, zeros_f32(128, 512))
            p3 = pm - p1
            ps, kt = [p1, p2, p3], T - 2
        elif T == 1:
            ps, kt = [p2, pm], 0
        else:
            ps, kt = [pm], 0
        outs = []
        for h in range(4):
            hs = slice(128 * h, 128 * h + 128)
            pp = jnp.concatenate([x[:, hs] for x in ps], axis=0).astype(BF)
            f0 = 64 * g + 16 * h
            vt = jnp.concatenate(
                [_bf(vtu[1, kt + j, f0:f0 + 16, :]) for j in range(len(ps))], axis=1)
            outs.append(_dot(vt, pp))
        finish(1, g, t, outs, inv)

    def a_valid(nk):
        r = lax.broadcasted_iota(jnp.int32, (nk, 512), 0)
        c = lax.broadcasted_iota(jnp.int32, (nk, 512), 1) & 127
        d = c - r + (nk - 128)
        return (d >= 0) & (d <= 14) & ((d & 1) == 0)

    def a_qk(i, g, t):
        T = 2 * i + t
        s_ref = next_slot()
        if T >= 1:
            s = _dot_nt(_bf(ku[0, g, 64 * T - 8:64 * T + 64, :]), qcat(0, g, t))
            s = jnp.where(a_valid(144), s, NEG)
            s_ref[0:144] = s
        else:
            s = _dot_nt(_bf(ku[0, g, 0:64, :]), qcat(0, g, t))
            s = jnp.where(a_valid(128), s, NEG)
            s_ref[0:128] = s
        m = jnp.max(s, axis=0, keepdims=True)
        return s_ref, m

    def a_pv(i, g, t, st):
        s_ref, m = st
        T = 2 * i + t
        nk = 144 if T >= 1 else 128
        p = jnp.exp2(s_ref[pl.ds(z8, nk)] - m)
        l = jnp.sum(p, axis=0, keepdims=True)
        inv = recip(l)
        outs = []
        for h in range(4):
            hs = slice(128 * h, 128 * h + 128)
            f0 = 64 * g + 16 * h
            if T >= 1:
                o = _dot(_bf(vtu[0, T, f0:f0 + 16, :]), p[16:144, hs].astype(BF))
                ph = jnp.concatenate([jnp.zeros((112, 128), BF), p[0:16, hs].astype(BF)], axis=0)
                o = o + _dot(_bf(vtu[0, T - 1, f0:f0 + 16, :]), ph)
            else:
                o = _dot(_bf(vtu[0, 0, f0:f0 + 16, :]), p[:, hs].astype(BF))
            outs.append(o)
        finish(0, g, t, outs, inv)

    qk = (a_qk, b_qk)
    pv = (a_pv, b_pv)

    out_copies = []
    for g in range(NG):
        proj_q(0, 0, g)
    for g in range(NG):
        proj_k(0, 0, g)
    for g in range(NG):
        proj_v(0, 0, g)

    NS = 2 * NB
    for s in range(NS):
        p, i = s % 2, s // 2
        pn, inx = (s + 1) % 2, (s + 1) // 2
        has_p = s + 1 < NS
        has_o = s >= 1
        po, io = (s - 1) % 2, (s - 1) // 2
        for g in range(NG):
            fill = []
            if has_p:
                fill += [lambda: proj_q(pn, inx, g), lambda: proj_k(pn, inx, g),
                         lambda: proj_v(pn, inx, g)]
            if has_o:
                fill += [lambda: out_copies.append(out_tile(po, io, g))]
            if SCHED == "a":
                if len(fill) >= 4:
                    f0, f1 = fill[:2], fill[2:]
                elif len(fill) == 3:
                    f0, f1 = fill[:2], fill[2:]
                else:
                    f0, f1 = [], fill
                st0 = qk[p](i, g, 0)
                for f in f0:
                    f()
                pv[p](i, g, 0, st0)
                st1 = qk[p](i, g, 1)
                for f in f1:
                    f()
                pv[p](i, g, 1, st1)
            elif SCHED == "b":
                st0 = qk[p](i, g, 0)
                st1 = qk[p](i, g, 1)
                for f in fill[:2]:
                    f()
                pv[p](i, g, 0, st0)
                for f in fill[2:]:
                    f()
                pv[p](i, g, 1, st1)
    for g in range(NG):
        out_copies.append(out_tile((NS - 1) % 2, (NS - 1) // 2, g))

    start_upto(len(copies))
    while state["waited"] < len(copies):
        copies[state["waited"]].wait()
        state["waited"] += 1
    for cp in out_copies:
        cp.wait()


N_IN_DMA = 2 * 32 + 2 * 8 * NB
N_OUT_DMA = 16 * NB


@jax.jit
def pallas_concat_heads__sliding_local_dilated__sliding_block__prompt_kernel(A_x, A_wqkv, A_wo, B_x, B_wqkv, B_wo):
    anyspec = pl.BlockSpec(memory_space=pl.ANY)
    out = pl.pallas_call(
        _kernel,
        in_specs=[anyspec] * 6,
        out_specs=anyspec,
        out_shape=jax.ShapeDtypeStruct((S, 2 * D), BF),
        scratch_shapes=[
            pltpu.VMEM((2, NB, 8, R, 128), BF),
            pltpu.VMEM((2, 32, D, 128), BF),
            pltpu.VMEM((2, NG, S, 128), BF),
            pltpu.VMEM((2, S // 128, D, 128), BF),
            pltpu.VMEM((2, NG, R, 128), BF),
            pltpu.VMEM((2, NG, R, 128), BF),
            pltpu.VMEM((16, S, 128), BF),
            pltpu.VMEM((8, 128), F32),
        ] + [pltpu.VMEM((256, 512), F32)] * NSLOT + [
            pltpu.SemaphoreType.DMA((N_IN_DMA,)),
            pltpu.SemaphoreType.DMA((N_OUT_DMA,)),
            pltpu.SemaphoreType.REGULAR,
        ],
        compiler_params=pltpu.CompilerParams(vmem_limit_bytes=100 * 2**20),
    )(A_x.reshape(S, D), A_wqkv, A_wo, B_x.reshape(S, D), B_wqkv, B_wo)
    return out.reshape(1, S, 2 * D)
```

```python
import jax
import jax.numpy as jnp
from jax import lax
import jax.experimental.pallas as pl
import jax.experimental.pallas.tpu as pltpu

S = 2048
D = 1024
DH = 32
R = 256
NB = S // R
NG = D // 128
LOG2E = 1.4426950408889634
QSCALE = (DH ** -0.5) * LOG2E
NEG = -1e30
NSLOT = 3
LOOKAHEAD = 6
SCHED = "a"
TICK = 250 * 1024
LEAD = 6
WGROUPS = [1, 1, 2, 4, 8, 8]
OBATCH = 2
PAIR = "cross"
XW = 2

BF = jnp.bfloat16
F32 = jnp.float32
U32 = jnp.uint32
NT = (((1,), (1,)), ((), ()))


def _dot(a, b):
    return jnp.dot(a, b, preferred_element_type=F32)


def _dot_nt(a, b):
    return lax.dot_general(a, b, NT, preferred_element_type=F32)


def _bf(x):
    return pltpu.bitcast(x, BF)


def _kernel(xa_hbm, wa_hbm, woa_hbm, xb_hbm, wb_hbm, wob_hbm, out_hbm,
            x_s, w_s, k_s, vt_s, q_s, o_s, out_s, zero_s, *rest):
    s_slots = rest[:NSLOT]
    in_sems, out_sems, zsem = rest[NSLOT:]
    x_hbm = (xa_hbm, xb_hbm)
    w_hbm = (wa_hbm, wb_hbm)
    wo_hbm = (woa_hbm, wob_hbm)

    copies = []
    index = {}

    cum = []

    def add(name, src, dst):
        index[name] = len(copies)
        copies.append(pltpu.make_async_copy(src, dst, in_sems.at[len(copies)]))
        nbytes = 2 * dst.shape[-1] * dst.shape[-2]
        cum.append((cum[-1] if cum else 0) + nbytes)

    def add_x(p, i):
        for k in range(8):
            add(("x", p, i, k), x_hbm[p].at[pl.ds(i * R, R), pl.ds(128 * k, 128)], x_s.at[p, i, k])

    def add_w(p, n):
        if n < 24:
            add(("w", p, n), w_hbm[p].at[:, pl.ds(128 * n, 128)], w_s.at[p, n])
        else:
            add(("w", p, n), wo_hbm[p].at[:, pl.ds(128 * (n - 24), 128)], w_s.at[p, n])

    add_x(0, 0)
    add_w(0, 0)
    add_x(0, 1)
    for n in range(1, 24):
        add_w(0, n)
    add_x(1, 0)
    for g in range(NG):
        for j in range(3):
            add_w(1, 8 * j + g)
    add_x(1, 1)
    if NB > 2:
        add_x(0, 2)
    for n in range(24, 32):
        add_w(0, n)
    if NB > 2:
        add_x(1, 2)
    for n in range(24, 32):
        add_w(1, n)
    for i in range(3, NB):
        add_x(0, i)
        add_x(1, i)

    state = {"started": 0, "waited": 0}

    def start_upto(n):
        n = min(n, len(copies))
        while state["started"] < n:
            copies[state["started"]].start()
            state["started"] += 1

    def tick(frac=1.0):
        state["budget"] += int(TICK * frac)
        n = state["started"]
        while n < len(copies) and cum[n] <= state["budget"]:
            n += 1
        start_upto(n)

    def need(name):
        j = index[name]
        start_upto(j + 1)
        while state["waited"] <= j:
            copies[state["waited"]].wait()
            state["waited"] += 1

    state["budget"] = 512 * 1024 + LEAD * 256 * 1024
    tick(0.0)

    xu = x_s.bitcast(U32)
    wu = w_s.bitcast(U32)
    ku = k_s.bitcast(U32)
    vtu = vt_s.bitcast(U32)
    qu = q_s.bitcast(U32)
    ou = o_s.bitcast(U32)

    zero_s[...] = jnp.zeros((8, 128), F32)
    z8 = pl.multiple_of(pl.semaphore_read(zsem), 8)
    zero_row = zero_s[pl.ds(z8, 8), :]

    def zeros_f32(r, c):
        return jnp.broadcast_to(zero_row[0:1, 0:1], (r, c))

    r128 = lax.broadcasted_iota(jnp.int32, (128, 512), 0)
    c128 = lax.broadcasted_iota(jnp.int32, (128, 512), 1) & 127
    upper = r128 > c128
    lane64 = lax.broadcasted_iota(jnp.int32, (64, 128), 1) >> 5

    def lhs_x(p, i):
        return jnp.concatenate([_bf(xu[p, i, k]) for k in range(8)], axis=1)

    def proj_tile(p, i, n):
        tick()
        return _dot(lhs_x(p, i), _bf(wu[p, n]))

    def proj_q(p, i, g):
        q_s[p, i % 3, g] = (proj_tile(p, i, g) * QSCALE).astype(BF)

    def proj_k(p, i, g):
        k_s[p, g, i * R:(i + 1) * R, :] = proj_tile(p, i, 8 + g).astype(BF)

    def proj_v(p, i, g):
        v = proj_tile(p, i, 16 + g)
        for t in range(R // 128):
            vt_s[p, 2 * i + t, 128 * g:128 * g + 128, :] = v[128 * t:128 * t + 128].T.astype(BF)

    def out_tile(p, i, n):
        tick()
        lhs = jnp.concatenate([_bf(ou[p, i, g]) for g in range(NG)], axis=1)
        out_s[8 * p + n, i * R:(i + 1) * R, :] = _dot(lhs, _bf(wu[p, 24 + n])).astype(BF)
        cps = []
        if (n + 1) % OBATCH == 0:
            for m in range(n + 1 - OBATCH, n + 1):
                cp = pltpu.make_async_copy(
                    out_s.at[8 * p + m, pl.ds(i * R, R), :],
                    out_hbm.at[pl.ds(i * R, R), pl.ds(D * p + 128 * m, 128)],
                    out_sems.at[(i * 2 + p) * 8 + m])
                cp.start()
                cps.append(cp)
        return cps

    def qcat(p, i, g, t):
        qi = qu[p, i % 3, g, 64 * t:64 * t + 64, :]
        return _bf(jnp.concatenate(
            [jnp.where(lane64 == h, qi, jnp.uint32(0)) for h in range(4)], axis=0))

    slot_ctr = {"n": 0}

    def next_slot():
        s = s_slots[slot_ctr["n"] % NSLOT]
        slot_ctr["n"] += 1
        return s

    def finish(p, i, g, t, outs, inv):
        o_t = jnp.concatenate(
            [outs[h] * inv[:, 128 * h:128 * h + 128] for h in range(4)], axis=0)
        o_s[p, i, g, 128 * t:128 * t + 128, :] = o_t.T.astype(BF)

    def recip(l):
        r0 = pl.reciprocal(l, approx=True)
        return r0 * (2.0 - l * r0)

    def b_qk(i, g, t):
        T = 2 * i + t
        tick(1.0)
        s_ref = next_slot()
        if T >= 2:
            k0 = (T - 2) * 64
            parts = []
            for j in range(8):
                parts.append(ku[1, g, k0 + 8 * j:k0 + 8 * j + 8, :])
                parts.append(ku[1, g, k0 + 128 + 8 * j:k0 + 128 + 8 * j + 8, :])
            parts.append(ku[1, g, k0 + 64:k0 + 128, :])
            s = _dot_nt(_bf(jnp.concatenate(parts, axis=0)), qcat(1, i, g, t))
            s1 = jnp.concatenate([s[32 * j:32 * j + 16] for j in range(8)], axis=0)
            s3 = jnp.concatenate([s[32 * j + 16:32 * j + 32] for j in range(8)], axis=0)
            sm = jnp.where(upper, s1, s3)
            s2 = s[256:384]
            m = jnp.max(jnp.maximum(sm, s2), axis=0, keepdims=True)
            s_ref[0:128] = sm
            s_ref[128:256] = s2
        elif T == 1:
            s = _dot_nt(_bf(ku[1, g, 0:128, :]), qcat(1, i, g, t))
            sm = jnp.where(upper, NEG, s[128:256])
            s2 = s[0:128]
            m = jnp.max(jnp.maximum(sm, s2), axis=0, keepdims=True)
            s_ref[0:128] = sm
            s_ref[128:256] = s2
        else:
            s = _dot_nt(_bf(ku[1, g, 0:64, :]), qcat(1, i, g, t))
            sm = jnp.where(upper, NEG, s)
            m = jnp.max(sm, axis=0, keepdims=True)
            s_ref[0:128] = sm
        return s_ref, m

    def b_pv(i, g, t, st):
        s_ref, m = st
        T = 2 * i + t
        pm = jnp.exp2(s_ref[pl.ds(z8, 128)] - m)
        if T >= 1:
            p2 = jnp.exp2(s_ref[pl.ds(z8 + 128, 128)] - m)
            l = jnp.sum(pm + p2, axis=0, keepdims=True)
        else:
            l = jnp.sum(pm, axis=0, keepdims=True)
        inv = recip(l)
        if T >= 2:
            p1 = jnp.where(upper, pm, zeros_f32(128, 512))
            p3 = pm - p1
            ps, kt = [p1, p2, p3], T - 2
        elif T == 1:
            ps, kt = [p2, pm], 0
        else:
            ps, kt = [pm], 0
        outs = []
        for h in range(4):
            hs = slice(128 * h, 128 * h + 128)
            pp = jnp.concatenate([x[:, hs] for x in ps], axis=0).astype(BF)
            f0 = 64 * g + 16 * h
            vt = jnp.concatenate(
                [_bf(vtu[1, kt + j, f0:f0 + 16, :]) for j in range(len(ps))], axis=1)
            outs.append(_dot(vt, pp))
        finish(1, i, g, t, outs, inv)

    def a_valid(nk):
        r = lax.broadcasted_iota(jnp.int32, (nk, 512), 0)
        c = lax.broadcasted_iota(jnp.int32, (nk, 512), 1) & 127
        d = c - r + (nk - 128)
        return (d >= 0) & (d <= 14) & ((d & 1) == 0)

    def a_qk(i, g, t):
        T = 2 * i + t
        tick(0.5)
        s_ref = next_slot()
        if T >= 1:
            s = _dot_nt(_bf(ku[0, g, 64 * T - 8:64 * T + 64, :]), qcat(0, i, g, t))
            s = jnp.where(a_valid(144), s, NEG)
            s_ref[0:144] = s
        else:
            s = _dot_nt(_bf(ku[0, g, 0:64, :]), qcat(0, i, g, t))
            s = jnp.where(a_valid(128), s, NEG)
            s_ref[0:128] = s
        m = jnp.max(s, axis=0, keepdims=True)
        return s_ref, m

    def a_pv(i, g, t, st):
        s_ref, m = st
        T = 2 * i + t
        nk = 144 if T >= 1 else 128
        p = jnp.exp2(s_ref[pl.ds(z8, nk)] - m)
        l = jnp.sum(p, axis=0, keepdims=True)
        inv = recip(l)
        outs = []
        for h in range(4):
            hs = slice(128 * h, 128 * h + 128)
            f0 = 64 * g + 16 * h
            if T >= 1:
                o = _dot(_bf(vtu[0, T, f0:f0 + 16, :]), p[16:144, hs].astype(BF))
                ph = jnp.concatenate([jnp.zeros((112, 128), BF), p[0:16, hs].astype(BF)], axis=0)
                o = o + _dot(_bf(vtu[0, T - 1, f0:f0 + 16, :]), ph)
            else:
                o = _dot(_bf(vtu[0, 0, f0:f0 + 16, :]), p[:, hs].astype(BF))
            outs.append(o)
        finish(0, i, g, t, outs, inv)

    qk = (a_qk, b_qk)
    pv = (a_pv, b_pv)

    out_copies = []
    starts, acc = {}, 0
    for gsz in WGROUPS:
        starts[acc] = acc + gsz - 1
        acc += gsz
    assert acc == 24
    for n in range(24):
        if n in starts:
            need(("w", 0, starts[n]))
            if n == 0:
                need(("x", 0, 1, 7))
        f = (proj_q, proj_k, proj_v)[n // 8]
        f(0, 0, n % 8)
        f(0, 1, n % 8)

    NS = 2 * NB
    o_at = {s: [] for s in range(NS)}
    for u in range(NS - 1):
        o_at[min(u + 3, NS - 1)].append(u)
    if NS >= 6:
        o_at[NS - 2] = [NS - 5, NS - 4]
        o_at[NS - 1] = [NS - 3, NS - 2]
        for s in range(NS - 2):
            o_at[s] = [u for u in o_at[s] if u < NS - 5]

    for s in range(NS):
        p, i = s % 2, s // 2
        if PAIR == "cross":
            pp, ip = (1, i) if p == 0 else (0, i + 2)
        elif s == 0:
            pp, ip = 1, 0
        else:
            pp, ip = p, i + 1
        has_p = ip < NB
        if XW and s == XW:
            need(("x", 1, NB - 1, 7))
        if has_p:
            need(("x", pp, ip, 7))
            if pp == 1 and ip == 0:
                need(("w", 1, 23))
        for u in o_at[s]:
            need(("w", u % 2, 31))
        for g in range(NG):
            fill = []
            if has_p:
                fill += [lambda: proj_q(pp, ip, g), lambda: proj_k(pp, ip, g),
                         lambda: proj_v(pp, ip, g)]
            for u in o_at[s]:
                fill += [lambda u=u: out_copies.extend(out_tile(u % 2, u // 2, g))]
            h = (len(fill) + 1) // 2
            st0 = qk[p](i, g, 0)
            for f in fill[:h]:
                f()
            pv[p](i, g, 0, st0)
            st1 = qk[p](i, g, 1)
            for f in fill[h:]:
                f()
            pv[p](i, g, 1, st1)
    need(("w", 1, 31))
    for g in range(NG):
        out_copies.extend(out_tile((NS - 1) % 2, (NS - 1) // 2, g))

    start_upto(len(copies))
    while state["waited"] < len(copies):
        copies[state["waited"]].wait()
        state["waited"] += 1
    for cp in out_copies:
        cp.wait()


N_IN_DMA = 2 * 32 + 2 * 8 * NB
N_OUT_DMA = 16 * NB


@jax.jit
def pallas_concat_heads__sliding_local_dilated__sliding_block__prompt_kernel(A_x, A_wqkv, A_wo, B_x, B_wqkv, B_wo):
    anyspec = pl.BlockSpec(memory_space=pl.ANY)
    out = pl.pallas_call(
        _kernel,
        in_specs=[anyspec] * 6,
        out_specs=anyspec,
        out_shape=jax.ShapeDtypeStruct((S, 2 * D), BF),
        scratch_shapes=[
            pltpu.VMEM((2, NB, 8, R, 128), BF),
            pltpu.VMEM((2, 32, D, 128), BF),
            pltpu.VMEM((2, NG, S, 128), BF),
            pltpu.VMEM((2, S // 128, D, 128), BF),
            pltpu.VMEM((2, 3, NG, R, 128), BF),
            pltpu.VMEM((2, NB, NG, R, 128), BF),
            pltpu.VMEM((16, S, 128), BF),
            pltpu.VMEM((8, 128), F32),
        ] + [pltpu.VMEM((256, 512), F32)] * NSLOT + [
            pltpu.SemaphoreType.DMA((N_IN_DMA,)),
            pltpu.SemaphoreType.DMA((N_OUT_DMA,)),
            pltpu.SemaphoreType.REGULAR,
        ],
        compiler_params=pltpu.CompilerParams(vmem_limit_bytes=100 * 2**20),
    )(A_x.reshape(S, D), A_wqkv, A_wo, B_x.reshape(S, D), B_wqkv, B_wo)
    return out.reshape(1, S, 2 * D)
```

```python
import jax
import jax.numpy as jnp
from jax import lax
import jax.experimental.pallas as pl
import jax.experimental.pallas.tpu as pltpu

S = 2048
D = 1024
DH = 32
R = 256
NTL = R // 128
NB = S // R
NG = D // 128
LOG2E = 1.4426950408889634
QSCALE = (DH ** -0.5) * LOG2E
NEG = -1e30
NSLOT = 3
TICK = 250 * 1024
LEAD = 6
WGROUPS = [1, 1, 2, 4, 8, 8]
OBATCH = 2

BF = jnp.bfloat16
F32 = jnp.float32
U32 = jnp.uint32
NT = (((1,), (1,)), ((), ()))


def _dot(a, b):
    return jnp.dot(a, b, preferred_element_type=F32)


def _dot_nt(a, b):
    return lax.dot_general(a, b, NT, preferred_element_type=F32)


def _bf(x):
    return pltpu.bitcast(x, BF)


def _kernel(xa_hbm, wa_hbm, woa_hbm, xb_hbm, wb_hbm, wob_hbm, out_hbm,
            x_s, w_s, k_s, vt_s, q_s, o_s, out_s, zero_s, *rest):
    s_slots = rest[:NSLOT]
    in_sems, out_sems, zsem = rest[NSLOT:]
    x_hbm = (xa_hbm, xb_hbm)
    w_hbm = (wa_hbm, wb_hbm)
    wo_hbm = (woa_hbm, wob_hbm)

    copies = []
    index = {}

    cum = []

    def add(name, src, dst):
        index[name] = len(copies)
        copies.append(pltpu.make_async_copy(src, dst, in_sems.at[len(copies)]))
        nbytes = 2 * dst.shape[-1] * dst.shape[-2]
        cum.append((cum[-1] if cum else 0) + nbytes)

    def add_x(p, i):
        for k in range(8):
            add(("x", p, i, k), x_hbm[p].at[pl.ds(i * R, R), pl.ds(128 * k, 128)], x_s.at[p, i, k])

    def add_w(p, n):
        if n < 24:
            add(("w", p, n), w_hbm[p].at[:, pl.ds(128 * n, 128)], w_s.at[p, n])
        else:
            add(("w", p, n), wo_hbm[p].at[:, pl.ds(128 * (n - 24), 128)], w_s.at[p, n])

    add_x(0, 0)
    add_w(0, 0)
    add_x(0, 1)
    for n in range(1, 24):
        add_w(0, n)
    add_x(1, 0)
    for g in range(NG):
        for j in range(3):
            add_w(1, 8 * j + g)
    add_x(1, 1)
    if NB > 2:
        add_x(0, 2)
    for n in range(24, 32):
        add_w(0, n)
    if NB > 2:
        add_x(1, 2)
    for n in range(24, 32):
        add_w(1, n)
    for i in range(3, NB):
        add_x(0, i)
        add_x(1, i)

    state = {"started": 0, "waited": 0}

    def start_upto(n):
        n = min(n, len(copies))
        while state["started"] < n:
            copies[state["started"]].start()
            state["started"] += 1

    def tick(frac=1.0):
        state["budget"] += int(TICK * frac)
        n = state["started"]
        while n < len(copies) and cum[n] <= state["budget"]:
            n += 1
        start_upto(n)

    def need(name):
        j = index[name]
        start_upto(j + 1)
        while state["waited"] <= j:
            copies[state["waited"]].wait()
            state["waited"] += 1

    state["budget"] = 2048 * R * 2 + LEAD * 256 * 1024
    tick(0.0)

    xu = x_s.bitcast(U32)
    wu = w_s.bitcast(U32)
    ku = k_s.bitcast(U32)
    vtu = vt_s.bitcast(U32)
    qu = q_s.bitcast(U32)
    ou = o_s.bitcast(U32)

    zero_s[...] = jnp.zeros((8, 128), F32)
    z8 = pl.multiple_of(pl.semaphore_read(zsem), 8)
    zero_row = zero_s[pl.ds(z8, 8), :]

    def zeros_f32(r, c):
        return jnp.broadcast_to(zero_row[0:1, 0:1], (r, c))

    r128 = lax.broadcasted_iota(jnp.int32, (128, 512), 0)
    c128 = lax.broadcasted_iota(jnp.int32, (128, 512), 1) & 127
    upper = r128 > c128
    lane64 = lax.broadcasted_iota(jnp.int32, (64, 128), 1) >> 5

    def lhs_x(p, i):
        return jnp.concatenate([_bf(xu[p, i, k]) for k in range(8)], axis=1)

    def proj_tile(p, i, n):
        tick()
        return _dot(lhs_x(p, i), _bf(wu[p, n]))

    def proj_q(p, i, g):
        q_s[p, i % 3, g] = (proj_tile(p, i, g) * QSCALE).astype(BF)

    def proj_k(p, i, g):
        k_s[p, g, i * R:(i + 1) * R, :] = proj_tile(p, i, 8 + g).astype(BF)

    def proj_v(p, i, g):
        v = proj_tile(p, i, 16 + g)
        for t in range(R // 128):
            vt_s[p, NTL * i + t, 128 * g:128 * g + 128, :] = v[128 * t:128 * t + 128].T.astype(BF)

    def out_tile(p, i, n):
        tick()
        lhs = jnp.concatenate([_bf(ou[p, i, g]) for g in range(NG)], axis=1)
        out_s[8 * p + n, i * R:(i + 1) * R, :] = _dot(lhs, _bf(wu[p, 24 + n])).astype(BF)
        cps = []
        if (n + 1) % OBATCH == 0:
            for m in range(n + 1 - OBATCH, n + 1):
                cp = pltpu.make_async_copy(
                    out_s.at[8 * p + m, pl.ds(i * R, R), :],
                    out_hbm.at[pl.ds(i * R, R), pl.ds(D * p + 128 * m, 128)],
                    out_sems.at[(i * 2 + p) * 8 + m])
                cp.start()
                cps.append(cp)
        return cps

    def qcat(p, i, g, t):
        qi = qu[p, i % 3, g, 64 * t:64 * t + 64, :]
        return _bf(jnp.concatenate(
            [jnp.where(lane64 == h, qi, jnp.uint32(0)) for h in range(4)], axis=0))

    slot_ctr = {"n": 0}

    def next_slot():
        s = s_slots[slot_ctr["n"] % NSLOT]
        slot_ctr["n"] += 1
        return s

    def finish(p, i, g, t, outs, inv):
        o_t = jnp.concatenate(
            [outs[h] * inv[:, 128 * h:128 * h + 128] for h in range(4)], axis=0)
        o_s[p, i, g, 128 * t:128 * t + 128, :] = o_t.T.astype(BF)

    def recip(l):
        r0 = pl.reciprocal(l, approx=True)
        return r0 * (2.0 - l * r0)

    lane32 = lax.broadcasted_iota(jnp.int32, (32, 128), 1) >> 5
    upper64 = (lax.broadcasted_iota(jnp.int32, (64, 256), 0)
               > (lax.broadcasted_iota(jnp.int32, (64, 256), 1) & 63))

    def b_qk(i, g, t):
        T = NTL * i + t
        tick(1.0)
        s_ref = next_slot()
        if T >= 2:
            ms = []
            for u in range(2):
                qi = qu[1, i % 3, g, 64 * t + 32 * u:64 * t + 32 * u + 32, :]
                order = (0, 1, 2, 3) if u == 0 else (1, 0, 3, 2)
                qm = _bf(jnp.concatenate(
                    [jnp.where(lane32 == h, qi, jnp.uint32(0)) for h in order], axis=0))
                k0 = (T - 2) * 64 + 32 * u
                parts = []
                for j in range(4):
                    parts.append(ku[1, g, k0 + 8 * j:k0 + 8 * j + 8, :])
                    parts.append(ku[1, g, k0 + 128 + 8 * j:k0 + 128 + 8 * j + 8, :])
                parts.append(ku[1, g, k0 + 32:k0 + 128, :])
                s = _dot_nt(_bf(jnp.concatenate(parts, axis=0)), qm)
                s1 = jnp.concatenate([s[32 * j:32 * j + 16] for j in range(4)], axis=0)
                s3 = jnp.concatenate([s[32 * j + 16:32 * j + 32] for j in range(4)], axis=0)
                sm = jnp.where(upper64, s1, s3)
                s2 = s[128:320]
                ms.append(jnp.maximum(jnp.max(sm, axis=0, keepdims=True),
                                      jnp.max(s2, axis=0, keepdims=True)))
                s_ref[0:64, 256 * u:256 * u + 256] = sm
                s_ref[64:256, 256 * u:256 * u + 256] = s2
            return s_ref, ms
        elif T == 1:
            s = _dot_nt(_bf(ku[1, g, 0:128, :]), qcat(1, i, g, t))
            sm = jnp.where(upper, NEG, s[128:256])
            s2 = s[0:128]
            m = jnp.max(jnp.maximum(sm, s2), axis=0, keepdims=True)
            s_ref[0:128] = sm
            s_ref[128:256] = s2
        else:
            s = _dot_nt(_bf(ku[1, g, 0:64, :]), qcat(1, i, g, t))
            sm = jnp.where(upper, NEG, s)
            m = jnp.max(sm, axis=0, keepdims=True)
            s_ref[0:128] = sm
        return s_ref, m

    def b_pv(i, g, t, st):
        s_ref, m = st
        T = NTL * i + t
        if T >= 2:
            pc = {}
            invs = []
            for u in range(2):
                us = slice(256 * u, 256 * u + 256)
                pm = jnp.exp2(s_ref[pl.ds(z8, 64), us] - m[u])
                p2 = jnp.exp2(s_ref[pl.ds(z8 + 64, 192), us] - m[u])
                l = jnp.sum(pm, axis=0, keepdims=True) + jnp.sum(p2, axis=0, keepdims=True)
                invs.append(recip(l))
                pf = jnp.where(upper64, pm, zeros_f32(64, 256))
                pc[u] = (pf, p2, pm - pf)
            lo64 = lax.broadcasted_iota(jnp.int32, (64, 128), 1) < 64
            lo128 = lax.broadcasted_iota(jnp.int32, (128, 128), 1) < 64
            outs = []
            for h in range(4):
                pi, odd = h // 2, h % 2
                hs = slice(128 * pi, 128 * pi + 128)
                f0_, m0_, l0_ = [x[:, hs] for x in pc[0]]
                f1_, m1_, l1_ = [x[:, hs] for x in pc[1]]
                z = zeros_f32(64, 128)
                sel = (lambda c, a, b: jnp.where(c, b, a)) if odd else (lambda c, a, b: jnp.where(c, a, b))
                pp = jnp.concatenate([
                    sel(lo64, f0_, z), sel(lo64, m0_[0:64], f1_),
                    sel(lo128, m0_[64:192], m1_[0:128]),
                    sel(lo64, l0_, m1_[128:192]), sel(lo64, z, l1_)], axis=0).astype(BF)
                f0 = 64 * g + 16 * h
                vt = jnp.concatenate(
                    [_bf(vtu[1, T - 2 + j, f0:f0 + 16, :]) for j in range(3)], axis=1)
                iv = sel(lo64[0:1], invs[0][:, hs], invs[1][:, hs])
                o = _dot(vt, pp) * iv
                outs.append(pltpu.roll(o, 64, 1) if odd else o)
            o_t = jnp.concatenate(outs, axis=0)
            o_s[1, i, g, 128 * t:128 * t + 128, :] = o_t.T.astype(BF)
            return
        pm = jnp.exp2(s_ref[pl.ds(z8, 128)] - m)
        if T >= 1:
            p2 = jnp.exp2(s_ref[pl.ds(z8 + 128, 128)] - m)
            l = jnp.sum(pm + p2, axis=0, keepdims=True)
        else:
            l = jnp.sum(pm, axis=0, keepdims=True)
        inv = recip(l)
        if T == 1:
            ps, kt = [p2, pm], 0
        else:
            ps, kt = [pm], 0
        outs = []
        for h in range(4):
            hs = slice(128 * h, 128 * h + 128)
            pp = jnp.concatenate([x[:, hs] for x in ps], axis=0).astype(BF)
            f0 = 64 * g + 16 * h
            vt = jnp.concatenate(
                [_bf(vtu[1, kt + j, f0:f0 + 16, :]) for j in range(len(ps))], axis=1)
            outs.append(_dot(vt, pp))
        finish(1, i, g, t, outs, inv)

    def a_valid(nk):
        r = lax.broadcasted_iota(jnp.int32, (nk, 256), 0)
        c = lax.broadcasted_iota(jnp.int32, (nk, 256), 1) & 63
        d = c - r + (nk - 64)
        return (d >= 0) & (d <= 14) & ((d & 1) == 0)

    lane32 = lax.broadcasted_iota(jnp.int32, (32, 128), 1) >> 5
    lane_lo = lax.broadcasted_iota(jnp.int32, (32, 128), 1) < 64

    def a_qk(i, g, t):
        T = NTL * i + t
        tick(0.4)
        s_ref = next_slot()
        ms = []
        for u in range(2):
            qi = qu[0, i % 3, g, 64 * t + 32 * u:64 * t + 32 * u + 32, :]
            order = (0, 1, 2, 3) if u == 0 else (1, 0, 3, 2)
            qm = _bf(jnp.concatenate(
                [jnp.where(lane32 == h, qi, jnp.uint32(0)) for h in order], axis=0))
            k1 = 64 * T + 32 * u + 32
            if T == 0 and u == 0:
                nk = 64
            else:
                nk = 80
            s = _dot_nt(_bf(ku[0, g, k1 - nk // 2:k1, :]), qm)
            s = jnp.where(a_valid(nk), s, NEG)
            s_ref[0:nk, 256 * u:256 * u + 256] = s
            ms.append(jnp.max(s, axis=0, keepdims=True))
        return s_ref, ms

    def a_pv(i, g, t, st):
        s_ref, ms = st
        T = NTL * i + t
        res = {}
        for u in range(2):
            halo = not (T == 0 and u == 0)
            nk = 80 if halo else 64
            p = jnp.exp2(s_ref[pl.ds(z8, nk), 256 * u:256 * u + 256] - ms[u])
            inv = recip(jnp.sum(p, axis=0, keepdims=True))
            for pi in range(2):
                hs = slice(128 * pi, 128 * pi + 128)
                f0 = 64 * g + 32 * pi
                vt = vtu[0, T, f0:f0 + 32, :]
                if u == 1:
                    pp = jnp.concatenate([jnp.zeros((48, 128), BF), p[:, hs].astype(BF)], axis=0)
                elif halo:
                    vt = jnp.where(lane_lo, vt, vtu[0, T - 1, f0:f0 + 32, :])
                    pp = jnp.concatenate([p[16:80, hs].astype(BF), jnp.zeros((48, 128), BF),
                                          p[0:16, hs].astype(BF)], axis=0)
                else:
                    pp = jnp.concatenate([p[:, hs].astype(BF), jnp.zeros((64, 128), BF)], axis=0)
                res[pi, u] = _dot(_bf(vt), pp) * inv[:, hs]
        outs = []
        for pi in range(2):
            r0, r1 = res[pi, 0], res[pi, 1]
            outs.append(jnp.where(lane_lo, r0[0:32], r1[0:32]))
            outs.append(pltpu.roll(jnp.where(lane_lo, r1[32:64], r0[32:64]), 64, 1))
        o_t = jnp.concatenate(outs, axis=0)
        o_s[0, i, g, 128 * t:128 * t + 128, :] = o_t.T.astype(BF)

    qk = (a_qk, b_qk)
    pv = (a_pv, b_pv)

    out_copies = []
    starts, acc = {}, 0
    for gsz in WGROUPS:
        starts[acc] = acc + gsz - 1
        acc += gsz
    assert acc == 24
    for n in range(24):
        if n in starts:
            need(("w", 0, starts[n]))
        f = (proj_q, proj_k, proj_v)[n // 8]
        f(0, 0, n % 8)
        if n == 0:
            need(("x", 0, 1, 7))
        f(0, 1, n % 8)

    NS = 2 * NB
    o_at = {s: [] for s in range(NS)}
    for u in range(NS - 1):
        o_at[min(u + 3, NS - 1)].append(u)
    if NS >= 6:
        o_at[NS - 2] = [NS - 5, NS - 4]
        o_at[NS - 1] = [NS - 3, NS - 2]
        for s in range(NS - 2):
            o_at[s] = [u for u in o_at[s] if u < NS - 5]

    for s in range(NS):
        p, i = s % 2, s // 2
        pp, ip = (1, i) if p == 0 else (0, i + 2)
        has_p = ip < NB
        if s >= 2 and s % 2 == 0:
            need(("x", 1, min(NB - 1, (s + 1) // 2 + 2), 7))
        if has_p:
            need(("x", pp, ip, 7))
            if pp == 1 and ip == 0:
                need(("w", 1, 23))
        for u in o_at[s]:
            need(("w", u % 2, 31))
        for g in range(NG):
            fill = []
            if has_p:
                fill += [lambda: proj_q(pp, ip, g), lambda: proj_k(pp, ip, g),
                         lambda: proj_v(pp, ip, g)]
            for u in o_at[s]:
                fill += [lambda u=u: out_copies.extend(out_tile(u % 2, u // 2, g))]
            cuts = [(len(fill) * t + NTL - 1) // NTL for t in range(NTL + 1)]
            sts = [qk[p](i, g, t) for t in range(NTL)]
            for t in range(NTL):
                for f in fill[cuts[t]:cuts[t + 1]]:
                    f()
                pv[p](i, g, t, sts[t])
    need(("w", 1, 31))
    for g in range(NG):
        out_copies.extend(out_tile((NS - 1) % 2, (NS - 1) // 2, g))

    start_upto(len(copies))
    while state["waited"] < len(copies):
        copies[state["waited"]].wait()
        state["waited"] += 1
    for cp in out_copies:
        cp.wait()


N_IN_DMA = 2 * 32 + 2 * 8 * NB
N_OUT_DMA = 16 * NB


@jax.jit
def pallas_concat_heads__sliding_local_dilated__sliding_block__prompt_kernel(A_x, A_wqkv, A_wo, B_x, B_wqkv, B_wo):
    anyspec = pl.BlockSpec(memory_space=pl.ANY)
    out = pl.pallas_call(
        _kernel,
        in_specs=[anyspec] * 6,
        out_specs=anyspec,
        out_shape=jax.ShapeDtypeStruct((S, 2 * D), BF),
        scratch_shapes=[
            pltpu.VMEM((2, NB, 8, R, 128), BF),
            pltpu.VMEM((2, 32, D, 128), BF),
            pltpu.VMEM((2, NG, S, 128), BF),
            pltpu.VMEM((2, S // 128, D, 128), BF),
            pltpu.VMEM((2, 3, NG, R, 128), BF),
            pltpu.VMEM((2, NB, NG, R, 128), BF),
            pltpu.VMEM((16, S, 128), BF),
            pltpu.VMEM((8, 128), F32),
        ] + [pltpu.VMEM((256, 512), F32)] * NSLOT + [
            pltpu.SemaphoreType.DMA((N_IN_DMA,)),
            pltpu.SemaphoreType.DMA((N_OUT_DMA,)),
            pltpu.SemaphoreType.REGULAR,
        ],
        compiler_params=pltpu.CompilerParams(vmem_limit_bytes=100 * 2**20),
    )(A_x.reshape(S, D), A_wqkv, A_wo, B_x.reshape(S, D), B_wqkv, B_wo)
    return out.reshape(1, S, 2 * D)
```
